```python
import jax
import jax.numpy as jnp

def _softmax(x, axis=-1):
    return jax.nn.softmax(x, axis=axis)
def _gelu(x):
    return jax.nn.gelu(x, approximate=True)
def _silu(x):
    return jax.nn.silu(x)
def _sigmoid(x):
    return jax.nn.sigmoid(x)
def _layernorm(x, axis=-1, eps=1e-5):
    m = jnp.mean(x, axis=axis, keepdims=True)
    v = jnp.var(x, axis=axis, keepdims=True)
    return (x - m) / jnp.sqrt(v + eps)
def _scatter_add(tgt, idx, src, axis=0):
    return tgt.at[idx].add(src)
def _segment_sum(src, seg, n):
    return jax.ops.segment_sum(src, seg, n)
class _Rng:
    def __init__(self, key):
        self._k = key
    def _next(self):
        self._k, sub = jax.random.split(self._k)
        return sub
    def normal(self, shape):
        return jax.random.normal(self._next(), shape, dtype=jnp.bfloat16)
    def randint(self, lo, hi, shape):
        return jax.random.randint(self._next(), shape, lo, hi, dtype=jnp.int32)
    def uniform(self, shape, lo=0.0, hi=1.0):
        return jax.random.uniform(self._next(), shape, jnp.bfloat16, lo, hi)
    def permutation(self, n):
        return jax.random.permutation(self._next(), n)


kernel_name = 'gated_mix__sliding_block_cached__glu_gated_swiglu__decode'

def setup_inputs():
    _rng = _Rng(jax.random.key(int.from_bytes(__import__("os").urandom(4), "little")))
    _w = (lambda a: (lambda t: t.astype(jnp.bfloat16) if jnp.issubdtype(t.dtype, jnp.floating) else t)(jnp.asarray(a)))
    def _A_setup():
        B, Sq, D = 1, 1, 640
        Hq, Hkv, Sk, Dh = 32, 32, 32768, 192
        assert Hq % Hkv == 0, (Hq, Hkv)
        return {
            "x": _w((lambda *s: _rng.normal(s) * 0.05)(B, Sq, D)),
            "k_cache": _w((lambda *s: _rng.normal(s) * 0.05)(B, Hkv, Sk, Dh)),
            "v_cache": _w((lambda *s: _rng.normal(s) * 0.05)(B, Hkv, Sk, Dh)),
            "wq": _w((lambda *s: _rng.normal(s) * 0.05)(D, Hq * Dh) * (D ** -0.5)),
            "wo": _w((lambda *s: _rng.normal(s) * 0.05)(Hq * Dh, D) * ((Hq * Dh) ** -0.5)),
        }
    _A_in = _A_setup()

    def _B_setup():
        B, S, D, F = 1, 1, 640, 1536
        return {
            "x": _w((lambda *s: _rng.normal(s) * 0.05)(B, S, D)),
            "w1": _w((lambda *s: _rng.normal(s) * 0.05)(D, F) * (2.0 / D) ** 0.5),
            "w3": _w((lambda *s: _rng.normal(s) * 0.05)(D, F) * (2.0 / D) ** 0.5),
            "w2": _w((lambda *s: _rng.normal(s) * 0.05)(F, D) * (2.0 / F) ** 0.5),
        }
    _B_in = _B_setup()

    return {
        "A_x": _A_in["x"],
        "A_k_cache": _A_in["k_cache"],
        "A_v_cache": _A_in["v_cache"],
        "A_wq": _A_in["wq"],
        "A_wo": _A_in["wo"],
        "B_x": _B_in["x"],
        "B_w1": _B_in["w1"],
        "B_w3": _B_in["w3"],
        "B_w2": _B_in["w2"],
        "gate_w": _w((lambda *s: _rng.normal(s) * 0.05)(640)),
    }

def reference(A_x, A_k_cache, A_v_cache, A_wq, A_wo, B_x, B_w1, B_w3, B_w2, gate_w):
    def _A_ref(x, k_cache, v_cache, wq, wo):
        B, Sq, D = x.shape
        Hq, Dh = 32, 192
        Hkv, Sk = k_cache.shape[1], k_cache.shape[2]
        W = min(4096, max(256, Sk // 4))
        rep = Hq // Hkv
        q = (lambda x, *d: x.transpose(*d))((x @ wq).reshape(B, Sq, Hq, Dh), 0, 2, 1, 3)
        k = jnp.repeat(k_cache[:, :, Sk - W:, :], rep, axis=1)
        v = jnp.repeat(v_cache[:, :, Sk - W:, :], rep, axis=1)
        scores = jnp.einsum("bhqd,bhkd->bhqk", q, k) * (Dh ** -0.5)
        p = _softmax(scores, axis=-1)
        o = jnp.einsum("bhqk,bhkd->bhqd", p, v)
        return (lambda x, *d: x.transpose(*d))(o, 0, 2, 1, 3).reshape(B, Sq, Hq * Dh) @ wo

    def _B_ref(x, w1, w3, w2):
        gate = jnp.einsum("bsd,df->bsf", x, w1)
        up = jnp.einsum("bsd,df->bsf", x, w3)
        h = _silu(gate) * up
        out = jnp.einsum("bsf,fd->bsd", h, w2)
        return out

    x = A_x
    g = _sigmoid((x * gate_w).sum(-1, keepdims=True))
    a = _A_ref(x, A_k_cache, A_v_cache, A_wq, A_wo)
    b = _B_ref(x, B_w1, B_w3, B_w2)
    return g * a + (1 - g) * b
```

```python
import jax
import jax.numpy as jnp
from jax import lax
import jax.experimental.pallas as pl
import jax.experimental.pallas.tpu as pltpu

_F32 = jnp.float32
_BF16 = jnp.bfloat16

_REGION = 256
_RUN = 4
_W_STEP = (2, 8)
_KV_STEP = (2, 10)
_AHEAD_W = 7
_AHEAD_KV = 6
_AHEAD_BG = 12
_NSEM = 16


def _as_tiles(w):
    R, C = w.shape
    n = (R // 8) * (C // 128)
    lead = n // _REGION if n % _REGION == 0 else 1
    return w.reshape(R // 8, 8, C // 128, 128).transpose(0, 2, 1, 3).reshape(lead, n // lead, 8, 128)


def _weight_steps(ntiles):
    runs = [(name, r, t) for t in range(0, _REGION, _RUN) for name, n in ntiles.items()
            for r in range(-(-n // _REGION)) if r * _REGION + t < n]

    def copies(rs):
        out = []
        for name, r, t in rs:
            if (out and ntiles[name] % _REGION == 0
                    and (out[-1][0], out[-1][1] + out[-1][2], out[-1][3]) == (name, r, t)):
                out[-1] = (name, out[-1][1], out[-1][2] + 1, t)
            else:
                out.append((name, r, 1, t))
        return out

    n0, n1 = _W_STEP
    nsteps, extra = divmod(len(runs), n0 + n1)
    steps, i = [], 0
    for s in range(nsteps):
        n = n0 + n1 + (1 if s < extra else 0)
        steps.append((copies(runs[i:i + n0]), copies(runs[i + n0:i + n])))
        i += n
    assert i == len(runs)
    return steps


def _column(row):
    return jnp.transpose(jnp.broadcast_to(row, (128, 128)))


def _aligned(i, n):
    return i if isinstance(i, int) else pl.multiple_of(i, n)


@jax.jit
def pallas_gated_mix__sliding_block_cached__glu_gated_swiglu__decode_kernel(
    A_x: jax.Array,
    A_k_cache: jax.Array,
    A_v_cache: jax.Array,
    A_wq: jax.Array,
    A_wo: jax.Array,
    B_x: jax.Array,
    B_w1: jax.Array,
    B_w3: jax.Array,
    B_w2: jax.Array,
    gate_w: jax.Array,
):
    del B_x
    B, Sq, D = A_x.shape
    _, H, SK, DH = A_k_cache.shape
    F = B_w1.shape[1]
    W = min(4096, max(256, SK // 4))
    assert B == 1 and Sq == 1 and A_wq.shape[1] == H * DH
    scale = DH ** -0.5

    CW = _RUN * 128
    NR = DH // 8
    NC = W // CW
    SR = sum(_KV_STEP)
    SPB = NR // SR
    SPH = 2 * NC * SPB
    assert W % CW == 0 and DH % (8 * SR) == 0 and DH == 192
    assert SPH % _NSEM == 0 and _AHEAD_BG <= min(_NSEM, SPH - 1)

    weights = dict(wq=A_wq, w1=B_w1, w3=B_w3, wo=A_wo, w2=B_w2)
    row_tiles = {name: w.shape[1] // 128 for name, w in weights.items()}
    ntiles = {name: w.size // 1024 for name, w in weights.items()}
    tiled = {name: _as_tiles(w) for name, w in weights.items()}
    kT = jnp.swapaxes(A_k_cache, 2, 3).reshape(H * DH, SK)
    vT = jnp.swapaxes(A_v_cache, 2, 3).reshape(H * DH, SK)

    def kv_step(h, j):
        m, c, r = j // (NC * SPB), (j // SPB) % NC, (j % SPB) * SR
        return ([("kv", h, m, c, r, _KV_STEP[0])], [("kv", h, m, c, r + _KV_STEP[0], _KV_STEP[1])])

    first = _weight_steps({name: ntiles[name] for name in ("wq", "w1", "w3")})
    last = _weight_steps({name: ntiles[name] for name in ("wo", "w2")})
    stream = first + [kv_step(h, j) for h in range(H) for j in range(SPH)] + last
    KV0, KV1, N = len(first), len(stream) - len(last), len(stream)
    ffn_steps = [1, 3, 6, 8, 11, 13, 17, 19, 22, 24, 26, 28]
    assert len(ffn_steps) == F // 128 and ffn_steps[-1] < SPH

    def kernel(x_ref, gw_ref, k_ref, v_ref, wq_ref, w1_ref, w3_ref, wo_ref, w2_ref, o_ref,
               kv_b, wq_b, w1_b, w3_b, wo_b, w2_b, x_b, gw_b, o_b,
               x_col, q_col, o_col, h_col, q_acc, g_acc, u_acc, s_s):
        src = dict(wq=wq_ref, w1=w1_ref, w3=w3_ref, wo=wo_ref, w2=w2_ref)
        dst = dict(wq=wq_b, w1=w1_b, w3=w3_b, wo=wo_b, w2=w2_b)

        def main(sems, small_sem):
            def copy(c, i):
                sem = sems.at[(i - KV0) % _NSEM]
                if c[0] == "kv":
                    _, h, m, cb, r, nr = c
                    return pltpu.make_async_copy(
                        (k_ref, v_ref)[m].at[pl.ds(_aligned(h * DH + r * 8, 8), nr * 8),
                                             pl.ds(SK - W + cb * CW, CW)],
                        kv_b.at[m, pl.ds(r * 8, nr * 8), pl.ds(cb * CW, CW)], sem)
                name, r, nr, t = c
                if ntiles[name] % _REGION == 0:
                    idx = (pl.ds(r, nr), pl.ds(t, _RUN))
                else:
                    idx = (0, pl.ds(r * _REGION + t, _RUN))
                return pltpu.make_async_copy(src[name].at[idx], dst[name].at[idx], sem)

            started = [0, 0]

            def start_until(prio, n):
                while started[prio] < min(n, N):
                    for c in stream[started[prio]][prio]:
                        copy(c, started[prio]).start(priority=prio)
                    started[prio] += 1

            def land(i):
                assert i < min(started)
                for c in stream[i][0] + stream[i][1]:
                    copy(c, i).wait()
                start_until(0, i + 1 + (_AHEAD_KV if KV0 - _AHEAD_W <= i < KV1 else _AHEAD_W))
                start_until(1, i + 1 + _AHEAD_BG)

            def weight_tiles(i):
                for name, r0, nr, t0 in stream[i][0] + stream[i][1]:
                    for r in range(r0, r0 + nr):
                        for t in range(t0, t0 + _RUN):
                            flat = r * _REGION + t
                            w = dst[name][r, t] if ntiles[name] % _REGION == 0 else dst[name][0, flat]
                            yield name, flat // row_tiles[name], flat % row_tiles[name], w.astype(_F32)

            small = [pltpu.make_async_copy(x_ref, x_b, small_sem),
                     pltpu.make_async_copy(gw_ref, gw_b, small_sem)]
            start_until(1, 1)
            for c in small:
                c.start()
            for i in range(_AHEAD_BG):
                start_until(0, min(i + 1, _AHEAD_W))
                start_until(1, i + 1)

            acc_refs = dict(wq=q_acc, w1=g_acc, w3=u_acc)
            written, done = set(), 0
            for i in range(KV0):
                land(i)
                if i == 0:
                    for c in small:
                        c.wait()
                if i < 2 * (D // 128):
                    if i % 2 == 0:
                        n0 = (i // 2) * 128
                        x_col[n0:n0 + 128, :] = _column(x_b[0, :, n0:n0 + 128].astype(_F32))
                elif i == 2 * (D // 128):
                    gate = jax.nn.sigmoid(jnp.sum(
                        x_b[0].astype(_F32) * gw_b[...].reshape(1, D).astype(_F32),
                        axis=-1, keepdims=True))
                else:
                    part = {}
                    for k in range(done, min(done + 2, i + 1)):
                        for name, a, b, w in weight_tiles(k):
                            y = w * x_col[a * 8:(a + 1) * 8, :]
                            part[name, b] = part[name, b] + y if (name, b) in part else y
                        done = k + 1
                    for (name, b), y in part.items():
                        if (name, b) in written:
                            acc_refs[name][b] += y
                        else:
                            acc_refs[name][b] = y
                            written.add((name, b))
            assert done == KV0

            def q_block(j):
                q = jnp.sum(q_acc[j], axis=0, keepdims=True) * scale
                q_col[pl.ds(_aligned(j * 128, 128), 128), :] = _column(q)

            def ffn_block(j):
                g = jnp.sum(g_acc[j], axis=0, keepdims=True)
                u = jnp.sum(u_acc[j], axis=0, keepdims=True)
                h_col[j * 128:(j + 1) * 128, :] = _column(g * jax.nn.sigmoid(g) * u * (1.0 - gate))

            def head(h, is_last):
                def rows(r):
                    return pl.ds(_aligned(h * DH + r * 8, 8), 8)

                mx = den = None
                s = p = None
                o = [None] * NR
                for j in range(SPH):
                    if is_last:
                        land(KV0 + h * SPH + j)
                    else:
                        for cs in kv_step(h, j):
                            copy(cs[0], KV0 + j).wait()
                        for prio, jn in ((0, j + _AHEAD_KV), (1, j + _AHEAD_BG)):
                            copy(kv_step(h + jn // SPH, jn % SPH)[prio][0], KV0 + jn).start(priority=prio)
                    m, c, r0 = j // (NC * SPB), (j // SPB) % NC, (j % SPB) * SR
                    if m == 0:
                        if r0 == 0:
                            s = [None] * _RUN
                        for r in range(r0, r0 + SR):
                            q = q_col[rows(r), :]
                            k = kv_b[0, r * 8:(r + 1) * 8, c * CW:(c + 1) * CW].astype(_F32)
                            for u in range(_RUN):
                                y = k[:, u * 128:(u + 1) * 128] * q
                                s[u] = y if s[u] is None else s[u] + y
                        if r0 + SR == NR:
                            for u in range(_RUN):
                                su = jnp.broadcast_to(jnp.sum(s[u], axis=0, keepdims=True), (8, 128))
                                s_s[_RUN * c + u] = su
                                mx = su if mx is None else jnp.maximum(mx, su)
                            if c == NC - 1:
                                mx = jnp.max(mx, axis=-1, keepdims=True)
                    else:
                        if r0 == 0:
                            p = [jnp.exp(s_s[_RUN * c + u] - mx) for u in range(_RUN)]
                            ps = (p[0] + p[1]) + (p[2] + p[3])
                            den = ps if den is None else den + ps
                            if c == NC - 1:
                                den = gate / jnp.sum(den, axis=-1, keepdims=True)
                        for r in range(r0, r0 + SR):
                            v = kv_b[1, r * 8:(r + 1) * 8, c * CW:(c + 1) * CW].astype(_F32)
                            y = [v[:, u * 128:(u + 1) * 128] * p[u] for u in range(_RUN)]
                            y = (y[0] + y[1]) + (y[2] + y[3])
                            o[r] = y if o[r] is None else o[r] + y
                            if c == NC - 1:
                                o_col[rows(r), :] = jnp.broadcast_to(
                                    jnp.sum(o[r], axis=-1, keepdims=True) * den, (8, 128))
                    if is_last:
                        if j in ffn_steps:
                            ffn_block(ffn_steps.index(j))
                    elif j in (SPH // 2 + 3, SPH // 2 + 5):
                        q_block((3 * (h + 1)) // 2 + (j - SPH // 2 - 3) // 2)

            q_block(0)
            q_block(1)
            assert started == [KV0 + _AHEAD_KV, KV0 + _AHEAD_BG]

            @pl.loop(0, H - 1)
            def _(h):
                head(h, False)

            started[0] += (H - 1) * SPH
            started[1] += (H - 1) * SPH
            head(H - 1, True)

            acc = [None] * (D // 128)
            for i in range(KV1, N):
                land(i)
                for name, a, b, w in weight_tiles(i):
                    y = w * (o_col if name == "wo" else h_col)[a * 8:(a + 1) * 8, :]
                    acc[b] = y if acc[b] is None else acc[b] + y
            assert started == [N, N]
            o_b[0] = jnp.concatenate([jnp.sum(a, axis=0, keepdims=True) for a in acc],
                                     axis=1).astype(o_b.dtype)
            out = pltpu.make_async_copy(o_b, o_ref, small_sem)
            out.start()
            out.wait()

        pl.run_scoped(main, pltpu.SemaphoreType.DMA((_NSEM,)), pltpu.SemaphoreType.DMA(()))

    hbm = pl.BlockSpec(memory_space=pl.ANY)
    return pl.pallas_call(
        kernel,
        out_shape=jax.ShapeDtypeStruct((B, Sq, D), A_x.dtype),
        in_specs=[hbm] * 9,
        out_specs=hbm,
        scratch_shapes=[
            pltpu.VMEM((2, DH, W), _BF16),
            *[pltpu.VMEM(t.shape, _BF16) for t in tiled.values()],
            pltpu.VMEM((1, 1, D), _BF16),
            pltpu.VMEM((D,), _BF16),
            pltpu.VMEM((1, 1, D), A_x.dtype),
            pltpu.VMEM((D, 128), _F32),
            pltpu.VMEM((H * DH, 128), _F32),
            pltpu.VMEM((H * DH, 128), _F32),
            pltpu.VMEM((F, 128), _F32),
            pltpu.VMEM((H * DH // 128, 8, 128), _F32),
            pltpu.VMEM((F // 128, 8, 128), _F32),
            pltpu.VMEM((F // 128, 8, 128), _F32),
            pltpu.VMEM((W // 128, 8, 128), _F32),
        ],
        compiler_params=pltpu.CompilerParams(vmem_limit_bytes=64 * 1024 * 1024),
    )(A_x, gate_w, kT, vT, *tiled.values())
```

```python
import jax
import jax.numpy as jnp
from jax import lax
import jax.experimental.pallas as pl
import jax.experimental.pallas.tpu as pltpu

_F32 = jnp.float32
_BF16 = jnp.bfloat16

_REGION = 256
_RUN = 4
_STEP = (1, 5)
_LAST_STEPS = ((0, 2), (0, 1))
_AHEAD = (13, 20)
_NSEM = 32
_FIRST_TILE = dict(wq=0, w1=192, w3=128, wo=0, w2=192)


def _as_tiles(w):
    R, C = w.shape
    n = (R // 8) * (C // 128)
    lead = n // _REGION if n % _REGION == 0 else 1
    return w.reshape(R // 8, 8, C // 128, 128).transpose(0, 2, 1, 3).reshape(lead, n // lead, 8, 128)


def _weight_steps(ntiles, last_steps=()):
    runs = []
    for t0 in range(0, _REGION, _RUN):
        for name, n in ntiles.items():
            t = (t0 + _FIRST_TILE[name]) % _REGION
            runs += [(name, r, t) for r in range(-(-n // _REGION)) if r * _REGION + t < n]

    def copies(rs):
        out = []
        for name, r, t in rs:
            if (out and ntiles[name] % _REGION == 0
                    and (out[-1][0], out[-1][1] + out[-1][2], out[-1][3]) == (name, r, t)):
                out[-1] = (name, out[-1][1], out[-1][2] + 1, t)
            else:
                out.append((name, r, 1, t))
        return out

    nsteps, extra = divmod(len(runs) - sum(a + b for a, b in last_steps), sum(_STEP))
    sizes = [(_STEP[0], _STEP[1] + (1 if s < extra else 0)) for s in range(nsteps)] + list(last_steps)
    steps, i = [], 0
    for a, b in sizes:
        steps.append((copies(runs[i:i + a]), copies(runs[i + a:i + a + b])))
        i += a + b
    assert i == len(runs) and i * _RUN == sum(ntiles.values())
    return steps


def _column(row):
    return jnp.transpose(jnp.broadcast_to(row, (128, 128)))


def _fold_lanes(y, op):
    y = [y[:, u * 128:(u + 1) * 128] for u in range(4)]
    return op(op(y[0], y[1]), op(y[2], y[3]))


def _aligned(i, n):
    return i if isinstance(i, int) else pl.multiple_of(i, n)


@jax.jit
def pallas_gated_mix__sliding_block_cached__glu_gated_swiglu__decode_kernel(
    A_x: jax.Array,
    A_k_cache: jax.Array,
    A_v_cache: jax.Array,
    A_wq: jax.Array,
    A_wo: jax.Array,
    B_x: jax.Array,
    B_w1: jax.Array,
    B_w3: jax.Array,
    B_w2: jax.Array,
    gate_w: jax.Array,
):
    del B_x
    B, Sq, D = A_x.shape
    _, H, SK, DH = A_k_cache.shape
    F = B_w1.shape[1]
    W = min(4096, max(256, SK // 4))
    assert B == 1 and Sq == 1 and A_wq.shape[1] == H * DH
    scale = DH ** -0.5

    CW = _RUN * 128
    NC = W // CW
    RB = 8 * sum(_STEP)
    NB = DH // RB
    SPH = 2 * NC * NB
    ND = D // 128
    assert _RUN == 4 and W % CW == 0 and DH % RB == 0 and DH == 192 and F // 128 <= H - 2
    assert SPH % _NSEM == 0 and _AHEAD[0] <= _AHEAD[1] <= _NSEM < SPH - 1

    weights = dict(wq=A_wq, w1=B_w1, w3=B_w3, wo=A_wo, w2=B_w2)
    row_tiles = {name: w.shape[1] // 128 for name, w in weights.items()}
    ntiles = {name: w.size // 1024 for name, w in weights.items()}
    tiled = {name: _as_tiles(w) for name, w in weights.items()}
    assert row_tiles["wq"] % _RUN == 0 and row_tiles["w1"] % _RUN == 0 and ND >= _RUN
    kT = jnp.swapaxes(A_k_cache, 2, 3).reshape(H * DH, SK)
    vT = jnp.swapaxes(A_v_cache, 2, 3).reshape(H * DH, SK)

    def kv_step(h, j):
        m, c, b = j // (NC * NB), (j // NB) % NC, j % NB + 1
        h, b = h + b // NB, b % NB
        if isinstance(h, int) and h == H:
            return [], []
        return [("kv", h, m, c, b, 0, _STEP[0])], [("kv", h, m, c, b, _STEP[0], _STEP[1])]

    def kv_slot(h, b):
        return b if b else (h % 2) * NB

    stream = _weight_steps({name: ntiles[name] for name in ("wq", "w1", "w3")})
    W_END = len(stream)
    stream += [kv_step(-1, (m * NC + c) * NB + NB - 1) for c in range(NC) for m in (0, 1)]
    KV_BEGIN = len(stream)
    stream += [kv_step(h, j) for h in range(H) for j in range(SPH)]
    KV_END = len(stream)
    stream += _weight_steps({name: ntiles[name] for name in ("wo", "w2")}, _LAST_STEPS)
    N = len(stream)
    position = [0]
    for high, background in stream[1:]:
        position.append(position[-1] + (1 if high or background else 0))
    q_steps = [SPH // 2 + 9, SPH // 2 + 17]
    ffn_step = SPH // 4 + 1

    def kernel(x_ref, gw_ref, k_ref, v_ref, wq_ref, w1_ref, w3_ref, wo_ref, w2_ref, o_ref,
               kv_b, wq_b, w1_b, w3_b, wo_b, w2_b, x_b, gw_b, o_b,
               x_col, q_col, o_col, h_col, q_acc, g_acc, u_acc, s_s):
        src = dict(wq=wq_ref, w1=w1_ref, w3=w3_ref, wo=wo_ref, w2=w2_ref)
        dst = dict(wq=wq_b, w1=w1_b, w3=w3_b, wo=wo_b, w2=w2_b)

        def weight_index(name, r, nr, t):
            if ntiles[name] % _REGION == 0:
                return pl.ds(r, nr), pl.ds(t, _RUN)
            return pl.ds(0, 1), pl.ds(r * _REGION + t, _RUN)

        def main(sems, small_sem):
            def copy(c, i):
                sem = sems.at[(i - KV_BEGIN) % _NSEM]
                if c[0] == "kv":
                    _, h, m, cb, b, r, nr = c
                    return pltpu.make_async_copy(
                        (k_ref, v_ref)[m].at[pl.ds(_aligned(h * DH + b * RB + r * 8, 8), nr * 8),
                                             pl.ds(SK - W + cb * CW, CW)],
                        kv_b.at[m, kv_slot(h, b), pl.ds(r * 8, nr * 8), pl.ds(cb * CW, CW)], sem)
                idx = weight_index(*c)
                return pltpu.make_async_copy(src[c[0]].at[idx], dst[c[0]].at[idx], sem)

            started = [0, 0]

            def start_next(prio):
                for c in stream[started[prio]][prio]:
                    copy(c, started[prio]).start(priority=prio)
                started[prio] += 1

            def land(i):
                assert i < min(started)
                for c in stream[i][0] + stream[i][1]:
                    copy(c, i).wait()
                for prio in (0, 1):
                    while started[prio] < N and position[started[prio]] <= position[i] + _AHEAD[prio]:
                        start_next(prio)
                assert max(started) <= i + 1 + _NSEM

            def weight_runs(i):
                for name, r0, nr, t in stream[i][0] + stream[i][1]:
                    w = dst[name][weight_index(name, r0, nr, t)].astype(_F32)
                    for r in range(nr):
                        yield (name, *divmod((r0 + r) * _REGION + t, row_tiles[name]), w[r])

            small = [pltpu.make_async_copy(x_ref, x_b, small_sem),
                     pltpu.make_async_copy(gw_ref, gw_b, small_sem)]
            start_next(1)
            for c in small:
                c.start()
            for i in range(_AHEAD[1]):
                for prio in (0, 1):
                    if started[prio] <= i < _AHEAD[prio]:
                        start_next(prio)

            acc_refs = dict(wq=q_acc, w1=g_acc, w3=u_acc)
            written, done = [], 0
            for i in range(W_END):
                land(i)
                n, phase = divmod(i - 2, 5)
                if n < ND:
                    if (n, phase) == (0, 0):
                        for c in small:
                            c.wait()
                    if n >= 0 and phase == 0:
                        x_col[n * 128:(n + 1) * 128, :] = _column(
                            x_b[0, :, n * 128:(n + 1) * 128].astype(_F32))
                elif (n, phase) == (ND, 0):
                    gate = jax.nn.sigmoid(jnp.sum(
                        x_b[0].astype(_F32) * gw_b[...].reshape(1, D).astype(_F32),
                        axis=-1, keepdims=True))
                else:
                    part = {}
                    for k in range(done, min(done + 2, i + 1)):
                        for name, a, b, w in weight_runs(k):
                            y = w * x_col[a * 8:(a + 1) * 8, :]
                            part[name, b] = part[name, b] + y if (name, b) in part else y
                        done = k + 1
                    for (name, b), y in part.items():
                        if (name, b) in written:
                            acc_refs[name][b:b + _RUN] += y
                        else:
                            acc_refs[name][b:b + _RUN] = y
                            written.append((name, b))
            assert done == W_END

            def q_block(j):
                q = jnp.sum(q_acc[j], axis=0, keepdims=True) * scale
                q_col[pl.ds(_aligned(j * 128, 128), 128), :] = _column(q)

            def ffn_block(j):
                g = jnp.sum(g_acc[j], axis=0, keepdims=True)
                u = jnp.sum(u_acc[j], axis=0, keepdims=True)
                h_col[pl.ds(_aligned(j * 128, 128), 128), :] = _column(
                    g * jax.nn.sigmoid(g) * u * (1.0 - gate))

            for i in range(W_END, KV_BEGIN):
                land(i)
                if i - W_END in (2, 8):
                    q_block((2, 8).index(i - W_END))

            def head(h):
                mx = den = s = p = None
                o = [None] * NB
                for j in range(SPH):
                    if isinstance(h, int):
                        land(KV_BEGIN + h * SPH + j)
                    else:
                        for cs in kv_step(h, j):
                            copy(cs[0], KV_BEGIN + j).wait()
                        for prio in (0, 1):
                            jn = j + _AHEAD[prio]
                            copy(kv_step(h + jn // SPH, jn % SPH)[prio][0],
                                 KV_BEGIN + jn).start(priority=prio)
                    m, c, b = j // (NC * NB), (j // NB) % NC, j % NB
                    rows = pl.ds(_aligned(h * DH + b * RB, 8), RB)
                    cols = pl.ds(c * CW, CW)
                    blk = kv_b[m, kv_slot(h, b), :, cols].astype(_F32)
                    if m == 0:
                        y = blk * jnp.concatenate([q_col[rows, :]] * _RUN, axis=1)
                        y = jnp.sum(y.reshape(RB // 8, 8, CW), axis=0)
                        s = y if b == 0 else s + y
                        if b == NB - 1:
                            s = jnp.broadcast_to(jnp.sum(s, axis=0, keepdims=True), (8, CW))
                            s_s[:, cols] = s
                            y = _fold_lanes(s, jnp.maximum)
                            mx = y if c == 0 else jnp.maximum(mx, y)
                            if c == NC - 1:
                                mx = jnp.max(mx, axis=-1, keepdims=True)
                    else:
                        if b == 0:
                            p = jnp.exp(s_s[:, cols] - mx)
                            y = _fold_lanes(p, jnp.add)
                            den = y if c == 0 else den + y
                            if c == NC - 1:
                                den = gate / jnp.sum(den, axis=-1, keepdims=True)
                        y = _fold_lanes((blk.reshape(RB // 8, 8, CW) * p).reshape(RB, CW), jnp.add)
                        o[b] = y if c == 0 else o[b] + y
                        if c == NC - 1:
                            o_col[rows, :] = jnp.broadcast_to(
                                jnp.sum(o[b], axis=-1, keepdims=True) * den[0:1], (RB, 128))
                    if j in q_steps and not (isinstance(h, int) and h == H - 1):
                        q_block(((h + 1) * DH) // 128 + q_steps.index(j))
                    elif j == ffn_step and not isinstance(h, int):
                        pl.when(h < F // 128)(lambda: ffn_block(h))

            assert started == [KV_BEGIN + _AHEAD[0], KV_BEGIN + _AHEAD[1]]
            lax.fori_loop(0, H - 2, lambda h, _: head(h), None)
            started[0] += (H - 2) * SPH
            started[1] += (H - 2) * SPH
            head(H - 2)
            head(H - 1)

            acc = [None] * ND
            for i in range(KV_END, N):
                land(i)
                for name, a, b, w in weight_runs(i):
                    col = o_col if name == "wo" else h_col
                    n = min(_RUN, ND - b)
                    ys = [w[:n] * col[a * 8:(a + 1) * 8, :]]
                    if n < _RUN:
                        ys.append(w[n:] * col[(a + 1) * 8:(a + 2) * 8, :])
                    for u in range(_RUN):
                        y = ys[0][u] if u < n else ys[1][u - n]
                        k = (b + u) % ND
                        acc[k] = y if acc[k] is None else acc[k] + y
            assert started == [N, N]
            o_b[0] = jnp.concatenate([jnp.sum(a, axis=0, keepdims=True) for a in acc],
                                     axis=1).astype(o_b.dtype)
            out = pltpu.make_async_copy(o_b, o_ref, small_sem)
            out.start()
            out.wait()

        pl.run_scoped(main, pltpu.SemaphoreType.DMA((_NSEM,)), pltpu.SemaphoreType.DMA(()))

    hbm = pl.BlockSpec(memory_space=pl.ANY)
    return pl.pallas_call(
        kernel,
        out_shape=jax.ShapeDtypeStruct((B, Sq, D), A_x.dtype),
        in_specs=[hbm] * 9,
        out_specs=hbm,
        scratch_shapes=[
            pltpu.VMEM((2, NB + 1, RB, W), _BF16),
            *[pltpu.VMEM(t.shape, _BF16) for t in tiled.values()],
            pltpu.VMEM((1, 1, D), _BF16),
            pltpu.VMEM((D,), _BF16),
            pltpu.VMEM((1, 1, D), A_x.dtype),
            pltpu.VMEM((D, 128), _F32),
            pltpu.VMEM((H * DH, 128), _F32),
            pltpu.VMEM((H * DH, 128), _F32),
            pltpu.VMEM((F, 128), _F32),
            pltpu.VMEM((H * DH // 128, 8, 128), _F32),
            pltpu.VMEM((F // 128, 8, 128), _F32),
            pltpu.VMEM((F // 128, 8, 128), _F32),
            pltpu.VMEM((8, W), _F32),
        ],
        compiler_params=pltpu.CompilerParams(vmem_limit_bytes=64 * 1024 * 1024),
    )(A_x, gate_w, kT, vT, *tiled.values())
```

```python
import jax
import jax.numpy as jnp
from jax import lax
import jax.experimental.pallas as pl
import jax.experimental.pallas.tpu as pltpu

_F32 = jnp.float32
_BF16 = jnp.bfloat16

_REGION = 256
_RUN = 4
_NPASS = _REGION // _RUN
_KV_STEP = (1, 5)
_AHEAD = (13, 17)
_NSEM = 32
_LATE = 7
_FIRST_TILE = dict(wq=0, w1=192, w3=128, wo=0, w2=192)


def _as_tiles(w):
    R, C = w.shape
    n = (R // 8) * (C // 128)
    lead = n // _REGION if n % _REGION == 0 else 1
    return w.reshape(R // 8, 8, C // 128, 128).transpose(0, 2, 1, 3).reshape(lead, n // lead, 8, 128)


def _pass_steps(ntiles, sizes):
    runs = [(name, r) for name, n in ntiles.items() for r in range(-(-n // _REGION))]

    def copies(rs):
        out = []
        for name, r in rs:
            if out and ntiles[name] % _REGION == 0 and out[-1][0] == name:
                out[-1] = (name, out[-1][1], out[-1][2] + 1)
            else:
                out.append((name, r, 1))
        return out

    steps, i = [], 0
    for a, b in sizes:
        steps.append((copies(runs[i:i + a]), copies(runs[i + a:i + a + b])))
        i += a + b
    assert i == len(runs)
    return steps


def _column(row):
    return jnp.transpose(jnp.broadcast_to(row, (128, 128)))


def _fold_lanes(y, op):
    y = [y[:, u * 128:(u + 1) * 128] for u in range(4)]
    return op(op(y[0], y[1]), op(y[2], y[3]))


def _aligned(i, n):
    return i if isinstance(i, int) else pl.multiple_of(i, n)


def _divmod(i, n):
    q = (i * -(-(1 << 16) // n)) >> 16
    return q, i - q * n


def _when(cond, fn):
    if not isinstance(cond, bool):
        pl.when(cond)(fn)
    elif cond:
        fn()


@jax.jit
def pallas_gated_mix__sliding_block_cached__glu_gated_swiglu__decode_kernel(
    A_x: jax.Array,
    A_k_cache: jax.Array,
    A_v_cache: jax.Array,
    A_wq: jax.Array,
    A_wo: jax.Array,
    B_x: jax.Array,
    B_w1: jax.Array,
    B_w3: jax.Array,
    B_w2: jax.Array,
    gate_w: jax.Array,
):
    del B_x
    B, Sq, D = A_x.shape
    _, H, SK, DH = A_k_cache.shape
    F = B_w1.shape[1]
    W = min(4096, max(256, SK // 4))
    assert B == 1 and Sq == 1 and A_wq.shape[1] == H * DH
    scale = DH ** -0.5

    CW = _RUN * 128
    NC = W // CW
    RB = 8 * sum(_KV_STEP)
    NB = DH // RB
    SPH = 2 * NC * NB
    ND = D // 128
    assert _RUN == 4 and W % CW == 0 and DH % RB == 0 and DH == 192 and F // 128 <= H - 2
    assert SPH % _NSEM == 0 and _AHEAD[0] <= _AHEAD[1] <= _NSEM < SPH - 1

    weights = dict(wq=A_wq, w1=B_w1, w3=B_w3, wo=A_wo, w2=B_w2)
    row_tiles = {name: w.shape[1] // 128 for name, w in weights.items()}
    ntiles = {name: w.size // 1024 for name, w in weights.items()}
    tiled = {name: _as_tiles(w) for name, w in weights.items()}
    assert row_tiles["wq"] % _RUN == 0 and row_tiles["w1"] % _RUN == 0
    kT = jnp.swapaxes(A_k_cache, 2, 3).reshape(H * DH, SK)
    vT = jnp.swapaxes(A_v_cache, 2, 3).reshape(H * DH, SK)

    in_tiles = {name: ntiles[name] for name in ("wq", "w1", "w3")}
    out_tiles = {name: ntiles[name] for name in ("wo", "w2")}
    in_steps = _pass_steps(in_tiles, ((1, 4), (1, 5), (1, 5), (1, 5)))
    out_steps = _pass_steps(out_tiles, ((1, 5), (1, 5), (1, 6)))
    end_steps = _pass_steps(out_tiles, ((1, 5), (1, 5), (1, 3), (0, 2), (0, 1)))

    def weight_step(steps):
        return lambda p, j: tuple([c + (p,) for c in cs] for cs in steps[j])

    def kv_step(h, j):
        m, c, b = j // (NC * NB), (j // NB) % NC, j % NB + 1
        h, b = h + b // NB, b % NB
        if isinstance(h, int) and h == H:
            return [], []
        return [("kv", h, m, c, b, 0, _KV_STEP[0])], [("kv", h, m, c, b, _KV_STEP[0], _KV_STEP[1])]

    def kv_slot(h, b):
        return b if b else (h & 1) * NB

    stream = [weight_step(in_steps)(p, j) for p in range(_NPASS) for j in range(len(in_steps))]
    IN_END = len(stream)
    stream += [kv_step(-1, (m * NC + c) * NB + NB - 1) for c in range(NC) for m in (0, 1)]
    KV_BEGIN = len(stream)
    stream += [kv_step(h, j) for h in range(H) for j in range(SPH)]
    KV_END = len(stream)
    stream += [weight_step(out_steps)(p, j) for p in range(_NPASS - 1) for j in range(len(out_steps))]
    stream += [weight_step(end_steps)(_NPASS - 1, j) for j in range(len(end_steps))]
    N = len(stream)
    position = [0]
    for high, background in stream[1:]:
        position.append(position[-1] + (1 if high or background else 0))
    q_steps = [SPH // 2 + 9, SPH // 2 + 17]
    ffn_step = SPH // 4 + 1

    def kernel(x_ref, gw_ref, k_ref, v_ref, wq_ref, w1_ref, w3_ref, wo_ref, w2_ref, o_ref,
               kv_b, wq_b, w1_b, w3_b, wo_b, w2_b, x_b, gw_b, o_b,
               x_col, q_col, o_col, h_col, q_acc, g_acc, u_acc, s_s):
        src = dict(wq=wq_ref, w1=w1_ref, w3=w3_ref, wo=wo_ref, w2=w2_ref)
        dst = dict(wq=wq_b, w1=w1_b, w3=w3_b, wo=wo_b, w2=w2_b)

        def weight_run(name, r, nr, p):
            t = (p * _RUN + _FIRST_TILE[name]) & (_REGION - 1)
            if ntiles[name] % _REGION == 0:
                return t, True, (pl.ds(r, nr), pl.ds(t, _RUN))
            exists = True if (r + 1) * _REGION <= ntiles[name] else r * _REGION + t < ntiles[name]
            first = r * _REGION + t
            if not isinstance(exists, bool):
                first = jnp.minimum(first, ntiles[name] - _RUN)
            return t, exists, (pl.ds(0, 1), pl.ds(first, _RUN))

        def main(sems, small_sem):
            def transfer(c, i, action):
                sem = sems.at[i & (_NSEM - 1)]
                if c[0] == "kv":
                    _, h, m, cb, b, r, nr = c
                    action(pltpu.make_async_copy(
                        (k_ref, v_ref)[m].at[pl.ds(_aligned(h * DH + b * RB + r * 8, 8), nr * 8),
                                             pl.ds(SK - W + cb * CW, CW)],
                        kv_b.at[m, kv_slot(h, b), pl.ds(r * 8, nr * 8), pl.ds(cb * CW, CW)], sem))
                else:
                    _, exists, idx = weight_run(*c)
                    _when(exists, lambda: action(
                        pltpu.make_async_copy(src[c[0]].at[idx], dst[c[0]].at[idx], sem)))

            started = [0, 0]

            def start_next(prio):
                for c in stream[started[prio]][prio]:
                    transfer(c, started[prio], lambda cp: cp.start(priority=prio))
                started[prio] += 1

            def land(i):
                assert i < min(started)
                for c in stream[i][0] + stream[i][1]:
                    transfer(c, i, lambda cp: cp.wait())
                for prio in (0, 1):
                    while started[prio] < N and position[started[prio]] <= position[i] + _AHEAD[prio]:
                        start_next(prio)
                assert max(started) <= i + 1 + _NSEM

            def repeat(body, step, begin, n, lo, hi, end, carry=None):
                def rolled(p, carry):
                    i0 = begin if n % _NSEM == 0 else begin + p * n

                    def land_step(j):
                        for cs in step(p, j):
                            for c in cs:
                                transfer(c, i0 + j, lambda cp: cp.wait())
                        for prio in (0, 1):
                            jn = j + _AHEAD[prio]
                            for c in step(p + jn // n, jn % n)[prio]:
                                transfer(c, i0 + jn, lambda cp: cp.start(priority=prio))
                    return body(p, land_step, carry)

                assert started == [begin + lo * n + a for a in _AHEAD]
                assert all(stream[begin + k] == step(k // n, k % n) and all(stream[begin + k])
                           for k in range(lo * n, hi * n + _AHEAD[1]))
                carry = lax.fori_loop(lo, hi, rolled, carry)
                started[0] += (hi - lo) * n
                started[1] += (hi - lo) * n
                for p in range(hi, end):
                    carry = body(p, lambda j: land(begin + p * n + j), carry)
                return carry

            small = [pltpu.make_async_copy(x_ref, x_b, small_sem),
                     pltpu.make_async_copy(gw_ref, gw_b, small_sem)]
            start_next(1)
            for c in small:
                c.start()
            for i in range(_AHEAD[1]):
                for prio in (0, 1):
                    if started[prio] <= i < _AHEAD[prio]:
                        start_next(prio)

            acc_refs = dict(wq=q_acc, w1=g_acc, w3=u_acc)
            for ref in acc_refs.values():
                ref[...] = jnp.zeros(ref.shape, _F32)
            x_steps = [2 + 5 * n for n in range(ND)]
            assert x_steps[-1] < _LATE * len(in_steps)
            for i in range(_LATE * len(in_steps)):
                land(i)
                if i == x_steps[0]:
                    for c in small:
                        c.wait()
                if i in x_steps:
                    n = x_steps.index(i) * 128
                    x_col[n:n + 128, :] = _column(x_b[0, :, n:n + 128].astype(_F32))
            gate = jax.nn.sigmoid(jnp.sum(
                x_b[0].astype(_F32) * gw_b[...].reshape(1, D).astype(_F32), axis=-1, keepdims=True))

            def project_in(p, j):
                for name, r0, nr in in_steps[j][0] + in_steps[j][1]:
                    t, exists, idx = weight_run(name, r0, nr, p)

                    def run():
                        w = dst[name][idx].astype(_F32)
                        part = {}
                        for r in range(nr):
                            a0, b0 = divmod((r0 + r) * _REGION, row_tiles[name])
                            a = a0 + _divmod(t + b0, row_tiles[name])[0]
                            y = w[r] * x_col[pl.ds(_aligned(a * 8, 8), 8), :]
                            part[b0] = part[b0] + y if b0 in part else y
                        at = {b0: pl.ds(_divmod(t + b0, row_tiles[name])[1], _RUN) for b0 in part}
                        part = {b0: y + acc_refs[name][at[b0]] for b0, y in part.items()}
                        for b0, y in part.items():
                            acc_refs[name][at[b0]] = y
                    _when(exists, run)

            def in_pass(p, land_step, _):
                for j in range(len(in_steps)):
                    land_step(j)
                    project_in(p - _LATE, j)

            n = len(in_steps)
            rolled_end = _NPASS - -(-_AHEAD[1] // n)
            repeat(in_pass, weight_step(in_steps), 0, n, _LATE, rolled_end, rolled_end)

            def q_block(j):
                q = jnp.sum(q_acc[j], axis=0, keepdims=True) * scale
                q_col[pl.ds(_aligned(j * 128, 128), 128), :] = _column(q)

            def ffn_block(j):
                g = jnp.sum(g_acc[j], axis=0, keepdims=True)
                u = jnp.sum(u_acc[j], axis=0, keepdims=True)
                h_col[pl.ds(_aligned(j * 128, 128), 128), :] = _column(
                    g * jax.nn.sigmoid(g) * u * (1.0 - gate))

            done = (rolled_end - _LATE) * n
            for i in range(rolled_end * n, KV_BEGIN):
                land(i)
                for k in range(done, min(done + 2, i + 1, IN_END)):
                    project_in(k // n, k % n)
                    done = k + 1
                if KV_BEGIN - i in (8, 3):
                    assert done == IN_END
                    q_block((8, 3).index(KV_BEGIN - i))

            def head(h, land_step, _):
                mx = den = s = p = None
                o = [None] * NB
                for j in range(SPH):
                    land_step(j)
                    m, c, b = j // (NC * NB), (j // NB) % NC, j % NB
                    rows = pl.ds(_aligned(h * DH + b * RB, 8), RB)
                    cols = pl.ds(c * CW, CW)
                    blk = kv_b[m, kv_slot(h, b), :, cols].astype(_F32)
                    if m == 0:
                        y = blk * jnp.concatenate([q_col[rows, :]] * _RUN, axis=1)
                        y = jnp.sum(y.reshape(RB // 8, 8, CW), axis=0)
                        s = y if b == 0 else s + y
                        if b == NB - 1:
                            s = jnp.broadcast_to(jnp.sum(s, axis=0, keepdims=True), (8, CW))
                            s_s[:, cols] = s
                            y = _fold_lanes(s, jnp.maximum)
                            mx = y if c == 0 else jnp.maximum(mx, y)
                            if c == NC - 1:
                                mx = jnp.max(mx, axis=-1, keepdims=True)
                    else:
                        if b == 0:
                            p = jnp.exp(s_s[:, cols] - mx)
                            y = _fold_lanes(p, jnp.add)
                            den = y if c == 0 else den + y
                            if c == NC - 1:
                                den = gate / jnp.sum(den, axis=-1, keepdims=True)
                        y = _fold_lanes((blk.reshape(RB // 8, 8, CW) * p).reshape(RB, CW), jnp.add)
                        o[b] = y if c == 0 else o[b] + y
                        if c == NC - 1:
                            o_col[rows, :] = jnp.broadcast_to(
                                jnp.sum(o[b], axis=-1, keepdims=True) * den[0:1], (RB, 128))
                    if j in q_steps and not (isinstance(h, int) and h == H - 1):
                        q_block((((h + 1) * DH) >> 7) + q_steps.index(j))
                    elif j == ffn_step:
                        _when(h < F // 128, lambda: ffn_block(h))

            repeat(head, kv_step, KV_BEGIN, SPH, 0, H - 2, H)

            def out_pass(steps, like):
                def body(p, land_step, acc):
                    acc = list(acc)
                    tile_row = [_divmod(p * _RUN + k, ND)[0] for k in range(ND)]
                    for j, (high, background) in enumerate(steps):
                        land_step(j)
                        for name, r0, nr in high + background:
                            t, exists, _ = weight_run(name, r0, nr, like)
                            if not exists:
                                continue
                            col = o_col if name == "wo" else h_col
                            w = dst[name][weight_run(name, r0, nr, p)[2]].astype(_F32)
                            for r in range(nr):
                                for u in range(_RUN):
                                    a0, k = divmod((r0 + r) * _REGION + t - like * _RUN + u, ND)
                                    rows = pl.ds(_aligned((a0 + tile_row[k]) * 8, 8), 8)
                                    acc[k] += w[r, u] * col[rows, :]
                    return tuple(acc[(k + _RUN) % ND] for k in range(ND))
                return body

            wrap = (_REGION - _FIRST_TILE["w2"]) // _RUN
            assert _FIRST_TILE["wo"] == 0 and _FIRST_TILE["w2"] == ntiles["w2"] % _REGION
            n = len(out_steps)
            acc = (jnp.zeros((8, 128), _F32),) * ND
            acc = repeat(out_pass(out_steps, 0), weight_step(out_steps), KV_END, n, 0, wrap, wrap, acc)
            acc = repeat(out_pass(out_steps, wrap), weight_step(out_steps), KV_END, n,
                         wrap, _NPASS - 1 - -(-_AHEAD[1] // n), _NPASS - 1, acc)
            acc = out_pass(end_steps, wrap)(_NPASS - 1, lambda j: land(N - len(end_steps) + j), acc)
            assert started == [N, N]
            o_b[0] = jnp.concatenate(
                [jnp.sum(acc[(b - _REGION) % ND], axis=0, keepdims=True) for b in range(ND)],
                axis=1).astype(o_b.dtype)
            out = pltpu.make_async_copy(o_b, o_ref, small_sem)
            out.start()
            out.wait()

        pl.run_scoped(main, pltpu.SemaphoreType.DMA((_NSEM,)), pltpu.SemaphoreType.DMA(()))

    hbm = pl.BlockSpec(memory_space=pl.ANY)
    return pl.pallas_call(
        kernel,
        out_shape=jax.ShapeDtypeStruct((B, Sq, D), A_x.dtype),
        in_specs=[hbm] * 9,
        out_specs=hbm,
        scratch_shapes=[
            pltpu.VMEM((2, NB + 1, RB, W), _BF16),
            *[pltpu.VMEM(t.shape, _BF16) for t in tiled.values()],
            pltpu.VMEM((1, 1, D), _BF16),
            pltpu.VMEM((D,), _BF16),
            pltpu.VMEM((1, 1, D), A_x.dtype),
            pltpu.VMEM((D, 128), _F32),
            pltpu.VMEM((H * DH, 128), _F32),
            pltpu.VMEM((H * DH, 128), _F32),
            pltpu.VMEM((F, 128), _F32),
            pltpu.VMEM((H * DH // 128, 8, 128), _F32),
            pltpu.VMEM((F // 128, 8, 128), _F32),
            pltpu.VMEM((F // 128, 8, 128), _F32),
            pltpu.VMEM((8, W), _F32),
        ],
        compiler_params=pltpu.CompilerParams(vmem_limit_bytes=64 * 1024 * 1024),
    )(A_x, gate_w, kT, vT, *tiled.values())
```
